```python
import os as _os
_os.environ.setdefault("JAX_PLATFORMS", "cpu")
import jax
import jax.numpy as jnp

def _softmax(x, axis=-1):
    return jax.nn.softmax(x, axis=axis)
def _gelu(x):
    return jax.nn.gelu(x, approximate=True)
def _silu(x):
    return jax.nn.silu(x)
def _sigmoid(x):
    return jax.nn.sigmoid(x)
def _layernorm(x, axis=-1, eps=1e-5):
    m = jnp.mean(x, axis=axis, keepdims=True)
    v = jnp.var(x, axis=axis, keepdims=True)
    return (x - m) / jnp.sqrt(v + eps)
def _scatter_add(tgt, idx, src, axis=0):
    return tgt.at[idx].add(src)
def _segment_sum(src, seg, n):
    return jax.ops.segment_sum(src, seg, n)
class _Rng:
    def __init__(self, key):
        self._k = key
    def _next(self):
        self._k, sub = jax.random.split(self._k)
        return sub
    def normal(self, shape):
        return jax.random.normal(self._next(), shape, dtype=jnp.bfloat16)
    def randint(self, lo, hi, shape):
        return jax.random.randint(self._next(), shape, lo, hi, dtype=jnp.int32)
    def uniform(self, shape, lo=0.0, hi=1.0):
        return jax.random.uniform(self._next(), shape, jnp.bfloat16, lo, hi)
    def permutation(self, n):
        return jax.random.permutation(self._next(), n)


kernel_name = 'gated_mix__linear_attn_block__mixer_s_mlp__prompt'

def setup_inputs():
    _rng = _Rng(jax.random.key(int.from_bytes(__import__("os").urandom(4), "little")))
    _w = (lambda a: (lambda t: t.astype(jnp.bfloat16) if jnp.issubdtype(t.dtype, jnp.floating) else t)(jnp.asarray(a)))
    def _A_setup():
        B, S, D = 1, 2048, 640
        return {
            "x": _w((lambda *s: _rng.normal(s) * 0.05)(B, S, D)),
            "wqkv": _w((lambda *s: _rng.normal(s) * 0.8)(D, 3 * D)),
            "wo": _w((lambda *s: _rng.normal(s) * 0.1)(D, D)),
        }
    _A_in = _A_setup()

    def _B_setup():
        B, S, D, F = 1, 2048, 640, 1728
        return {
            "x":  _w((lambda *s: _rng.normal(s) * 0.05)(B, S, D)),
            "w1": _w((lambda *s: _rng.normal(s) * 0.2)(D, D) * (D ** -0.5)),
            "w2": _w((lambda *s: _rng.normal(s) * 0.2)(D, D) * (D ** -0.5)),
            "w3": _w((lambda *s: _rng.normal(s) * 0.2)(D, F) * (D ** -0.5)),
            "w4": _w((lambda *s: _rng.normal(s) * 0.2)(F, D) * (F ** -0.5)),
        }
    _B_in = _B_setup()

    return {
        "A_x": _A_in["x"],
        "A_wqkv": _A_in["wqkv"],
        "A_wo": _A_in["wo"],
        "B_x": _B_in["x"],
        "B_w1": _B_in["w1"],
        "B_w2": _B_in["w2"],
        "B_w3": _B_in["w3"],
        "B_w4": _B_in["w4"],
        "gate_w": _w((lambda *s: _rng.normal(s) * 0.05)(640) * 16.0),
    }

def reference(A_x, A_wqkv, A_wo, B_x, B_w1, B_w2, B_w3, B_w4, gate_w):
    def _A_ref(x, wqkv, wo):
        B, S, D = x.shape
        H = 32; Dh = D // H
        qkv = (lambda x, *d: x.transpose(*d))((x @ wqkv).reshape(B, S, 3, H, Dh), 2, 0, 3, 1, 4)
        q, k, v = qkv[0], qkv[1], qkv[2]
        phi = lambda t: jnp.where(t > 0, t + 1, jnp.exp(t)) + 1e-6
        pq, pk = phi(q), phi(k)
        kv = jnp.einsum("bhsd,bhse->bhde", pk, v)
        z = jnp.einsum("bhsd->bhd", pk)
        num = jnp.einsum("bhqd,bhde->bhqe", pq, kv)
        den = jnp.einsum("bhqd,bhd->bhq", pq, z)[..., None] + 1e-6
        o = num / den
        return (lambda x, *d: x.transpose(*d))(o, 0, 2, 1, 3).reshape(B, S, D) @ wo

    def _B_ref(x, w1, w2, w3, w4):
        B, S, D = x.shape
        h = _gelu(_layernorm(x, axis=-1) @ w1)
        c = D // 4
        g0 = jnp.pad(h[:, :, 0*c:1*c], ((0, 0), (1, 0), (0, 0)))[:, :S, :]
        g1 = jnp.pad(h[:, :, 1*c:2*c], ((0, 0), (0, 1), (0, 0)))[:, 1:, :]
        g2 = jnp.pad(h[:, :, 2*c:3*c], ((0, 0), (2, 0), (0, 0)))[:, :S, :]
        g3 = jnp.pad(h[:, :, 3*c:   ], ((0, 0), (0, 2), (0, 0)))[:, 2:, :]
        hs = jnp.concatenate([g0, g1, g2, g3], axis=-1) @ w2
        x1 = x + hs
        h2 = _gelu(_layernorm(x1, axis=-1) @ w3) @ w4
        return x1 + h2

    x = A_x
    g = _sigmoid((x * gate_w).sum(-1, keepdims=True))
    a = _A_ref(x, A_wqkv, A_wo)
    b = _B_ref(x, B_w1, B_w2, B_w3, B_w4)
    return g * a + (1 - g) * b
```

```python
import functools
import jax
import jax.numpy as jnp
from jax import lax
import jax.experimental.pallas as pl
import jax.experimental.pallas.tpu as pltpu

S, D, F, H = 2048, 640, 1728, 32
DH = D // H
NT = (((1,), (1,)), ((), ()))
f32 = jnp.float32
bf16 = jnp.bfloat16
LO = (0, 112, 240, 368, 496)
HI = (144, 272, 400, 528, 640)


def _phi(t):
    return jnp.where(t > 0, t + 1.0, jnp.exp(t)) + 1e-6


def _gelu(x):
    c = 0.7978845608028654
    return 0.5 * x * (1.0 + jnp.tanh(c * (x + 0.044715 * (x * x * x))))


def _ln(x):
    m = jnp.mean(x, axis=-1, keepdims=True)
    xc = x - m
    v = jnp.mean(xc * xc, axis=-1, keepdims=True)
    return xc * lax.rsqrt(v + 1e-5)


def _dot(a, b):
    return jnp.dot(a, b, preferred_element_type=f32)


def _dot_nt(a, b):
    return lax.dot_general(a, b, NT, preferred_element_type=f32)


def make(BM1=256, BM2=256, U1=False, U2=False, PAD=8, XB=256):
    NB1 = S // BM1
    NB2 = S // BM2
    NX = S // XB

    def kernel(ax_hbm, wqkv_hbm, wo_hbm, bx_hbm, w1_hbm, w2_hbm, w3_hbm, w4_hbm, gw_ref,
               out_hbm,
               ax, wq, wk, wv, wo, w1, w2, w3, w4,
               wqT, wkT, P, Pb, zacc, zb, hbuf, Mf, Mb, obuf,
               sem_ax, sem_w, sem_o):
        def xcopy(i):
            return pltpu.make_async_copy(ax_hbm.at[0, pl.ds(i * XB, XB), :], ax.at[pl.ds(i * XB, XB), :], sem_ax.at[i])

        wcopies = dict(
            wk=pltpu.make_async_copy(wqkv_hbm.at[:, pl.ds(D, D)], wk, sem_w.at[0]),
            w1=pltpu.make_async_copy(w1_hbm, w1, sem_w.at[1]),
            wq=pltpu.make_async_copy(wqkv_hbm.at[:, pl.ds(0, D)], wq, sem_w.at[2]),
            wv=pltpu.make_async_copy(wqkv_hbm.at[:, pl.ds(2 * D, D)], wv, sem_w.at[3]),
            wo=pltpu.make_async_copy(wo_hbm, wo, sem_w.at[4]),
            w2=pltpu.make_async_copy(w2_hbm, w2, sem_w.at[5]),
            w3=pltpu.make_async_copy(w3_hbm, w3, sem_w.at[6]),
            w4=pltpu.make_async_copy(w4_hbm, w4, sem_w.at[7]),
        )
        wcopies["wk"].start()
        xcopy(0).start()
        wcopies["w1"].start()
        for i in range(1, NX):
            xcopy(i).start()
        for n in ("wq", "wv", "wo", "w2", "w3", "w4"):
            wcopies[n].start()

        P[...] = jnp.zeros_like(P)
        Mf[...] = jnp.zeros_like(Mf)
        zacc[...] = jnp.zeros_like(zacc)
        hbuf[:, 0:PAD, :] = jnp.zeros((5, PAD, 128), f32)
        hbuf[:, PAD + S:PAD + S + PAD, :] = jnp.zeros((5, PAD, 128), f32)

        wcopies["wk"].wait()
        wkT[...] = wk[...].T
        wcopies["w1"].wait()

        def phase1(i, carry):
            r0 = pl.multiple_of(i * BM1, BM1)
            for j in range(BM1 // XB):
                xcopy(i * (BM1 // XB) + j).wait()
            xa = ax[pl.ds(r0, BM1), :]
            kT = _dot_nt(wkT[...], xa)
            hpre = _dot(_ln(xa.astype(f32)).astype(bf16), w1[...])
            pkT = _phi(kT)
            zs = pkT[:, 0:128]
            for j in range(1, BM1 // 128):
                zs = zs + pkT[:, j * 128:(j + 1) * 128]
            zacc[...] += zs
            P[...] += _dot(pkT.astype(bf16), xa)
            h = _gelu(hpre)
            for t in range(5):
                hbuf[t, pl.ds(r0 + PAD, BM1), :] = h[:, t * 128:(t + 1) * 128]
            return carry

        if U1:
            for i in range(NB1):
                phase1(i, 0)
        else:
            lax.fori_loop(0, NB1, phase1, 0)

        wcopies["wv"].wait()
        wcopies["wo"].wait()
        wcopies["wq"].wait()
        wqT[...] = wq[...].T
        z = jnp.sum(zacc[...], axis=1, keepdims=True)
        zb[...] = jnp.broadcast_to(z, (D, 128))
        Pb[...] = P[...].astype(bf16)
        kvs = []
        for t in range(5):
            lo, hi = LO[t], HI[t]
            kvt = _dot(Pb[lo:hi, :], wv[:, t * 128:(t + 1) * 128])
            rh = (lax.broadcasted_iota(jnp.int32, (hi - lo, 128), 0) + lo) // DH
            ch = (lax.broadcasted_iota(jnp.int32, (hi - lo, 128), 1) + t * 128) // DH
            kvs.append(jnp.where(rh == ch, kvt, 0.0).astype(bf16))
        for t in range(5):
            lo, hi = LO[t], HI[t]
            Mf[lo:hi, :] += _dot(kvs[t], wo[t * 128:(t + 1) * 128, :])
        Mb[...] = Mf[...].astype(bf16)
        wcopies["w2"].wait()
        wcopies["w3"].wait()
        wcopies["w4"].wait()

        gw = gw_ref[...].reshape(1, D).astype(f32)

        def ocopy(i):
            return pltpu.make_async_copy(obuf.at[pl.ds(i * BM2, BM2), :], out_hbm.at[0, pl.ds(i * BM2, BM2), :], sem_o.at[i])

        def phase2(i, carry):
            BM = BM2
            r0 = pl.multiple_of(i * BM, BM)
            xa = ax[pl.ds(r0, BM), :]
            qT = _dot_nt(wqT[...], xa)

            def hload(t, off):
                return hbuf[t, pl.ds(r0 + PAD + off, BM), :]
            lane = lax.broadcasted_iota(jnp.int32, (BM, 128), 1)
            s0 = hload(0, -1)
            s1 = jnp.where(lane < 32, hload(1, -1), hload(1, 1))
            s2 = jnp.where(lane < 64, hload(2, 1), hload(2, -2))
            s3 = jnp.where(lane < 96, hload(3, -2), hload(3, 2))
            s4 = hload(4, 2)
            hsft = jnp.concatenate([s0, s1, s2, s3, s4], axis=1).astype(bf16)
            hs = _dot(hsft, w2[...])

            pqT = _phi(qT)
            zbv = zb[...]
            zfull = jnp.concatenate([zbv] * (BM // 128), axis=1)
            prod = (pqT * zfull).reshape(H // 2, 40, BM)
            sub = lax.broadcasted_iota(jnp.int32, (H // 2, 40, BM), 1)
            denA = jnp.sum(jnp.where(sub < 20, prod, 0.0), axis=1, keepdims=True) + 1e-6
            denB = jnp.sum(jnp.where(sub >= 20, prod, 0.0), axis=1, keepdims=True) + 1e-6
            rden = jnp.where(sub < 20, 1.0 / denA, 1.0 / denB)
            pqsT = (pqT.reshape(H // 2, 40, BM) * rden).reshape(D, BM)
            pqs = pqsT.astype(bf16).T
            a = _dot(pqs, Mb[...])

            xf = xa.astype(f32)
            x1 = xf + hs
            t = _gelu(_dot_nt(_ln(x1).astype(bf16), w3[...])).astype(bf16)
            h2 = _dot(t, w4[...])
            gl = jnp.sum(xf * gw, axis=-1, keepdims=True)
            g = jax.nn.sigmoid(gl)
            b = x1 + h2
            obuf[pl.ds(r0, BM), :] = (g * a + (1.0 - g) * b).astype(bf16)
            ocopy(i).start()
            return carry

        if U2:
            for i in range(NB2):
                phase2(i, 0)
        else:
            lax.fori_loop(0, NB2, phase2, 0)
        for i in range(NB2):
            ocopy(i).wait()

    @jax.jit
    def run(A_x, A_wqkv, A_wo, B_x, B_w1, B_w2, B_w3, B_w4, gate_w):
        any_spec = pl.BlockSpec(memory_space=pltpu.HBM)
        return pl.pallas_call(
            kernel,
            out_shape=jax.ShapeDtypeStruct((1, S, D), bf16),
            in_specs=[any_spec] * 8 + [pl.BlockSpec(memory_space=pltpu.VMEM)],
            out_specs=any_spec,
            scratch_shapes=[
                pltpu.VMEM((S, D), bf16),
                pltpu.VMEM((D, D), bf16), pltpu.VMEM((D, D), bf16), pltpu.VMEM((D, D), bf16), pltpu.VMEM((D, D), bf16),
                pltpu.VMEM((D, D), bf16), pltpu.VMEM((D, D), bf16), pltpu.VMEM((F, D), bf16), pltpu.VMEM((F, D), bf16),
                pltpu.VMEM((D, D), bf16), pltpu.VMEM((D, D), bf16),
                pltpu.VMEM((D, D), f32), pltpu.VMEM((D, D), bf16), pltpu.VMEM((D, 128), f32), pltpu.VMEM((D, 128), f32),
                pltpu.VMEM((5, S + 2 * PAD, 128), f32), pltpu.VMEM((D, D), f32), pltpu.VMEM((D, D), bf16), pltpu.VMEM((S, D), bf16),
                pltpu.SemaphoreType.DMA((NX,)),
                pltpu.SemaphoreType.DMA((8,)), pltpu.SemaphoreType.DMA((NB2,)),
            ],
            compiler_params=pltpu.CompilerParams(vmem_limit_bytes=100 * 1024 * 1024),
            name="gated_mix",
        )(A_x, A_wqkv, A_wo, B_x, B_w1, B_w2, B_w3.T, B_w4, gate_w)
    return run


_run = make()


def pallas_gated_mix__linear_attn_block__mixer_s_mlp__prompt_kernel(A_x, A_wqkv, A_wo, B_x, B_w1, B_w2, B_w3, B_w4, gate_w):
    return _run(A_x, A_wqkv, A_wo, B_x, B_w1, B_w2, B_w3, B_w4, gate_w)
```

```python
import contextlib
import jax
import jax.numpy as jnp
from jax import lax
import jax.experimental.pallas as pl
import jax.experimental.pallas.tpu as pltpu

S, D, F, H = 2048, 640, 1728, 32
DH = D // H
NT = (((1,), (1,)), ((), ()))
f32 = jnp.float32
bf16 = jnp.bfloat16
LO = (0, 112, 240, 368, 496)
HI = (144, 272, 400, 528, 640)


def _phi(t):
    return jnp.where(t > 0, t + 1.0, jnp.exp(t)) + 1e-6


def _ln(x):
    m = jnp.mean(x, axis=-1, keepdims=True)
    xc = x - m
    v = jnp.mean(xc * xc, axis=-1, keepdims=True)
    rs = lax.rsqrt(v + 1e-5)
    return x * rs - m * rs


def _gelu_scaled(x, half):
    c = 0.7978845608028654
    inner = x * (c + (c * 0.044715) * (x * x))
    return (half * x) * (1.0 + jnp.tanh(inner))


def _dot(a, b):
    return jnp.dot(a, b, preferred_element_type=f32)


def _dot_nt(a, b):
    return lax.dot_general(a, b, NT, preferred_element_type=f32)


def make(BM=256, PAD=8, UN2=2, SPLIT_OUT=True, FREM=True, scopes=False):
    NB = S // BM
    PEEL = 2

    def scope(name):
        return jax.named_scope(name) if scopes else contextlib.nullcontext()

    def kernel(ax_hbm, wqkv_hbm, wo_hbm, bx_hbm, w1_hbm, w2_hbm, w3_hbm, w4_hbm, gw_hbm,
               out_hbm,
               ax, wq, wk, wv, wo, w1, w2, w3, w5, gwv,
               wqT, P, zacc, zb, hbuf, obuf, gcol, grow,
               sem_ax, sem_wk, sem_w, sem_o):
        def xcopy(i):
            return pltpu.make_async_copy(ax_hbm.at[0, pl.ds(i * BM, BM), :], ax.at[pl.ds(i * BM, BM), :], sem_ax.at[i])

        wkcopy = pltpu.make_async_copy(wqkv_hbm.at[:, pl.ds(D, D)], wk, sem_wk.at[0])

        wcopies = dict(
            gw=pltpu.make_async_copy(gw_hbm, gwv, sem_w.at[0]),
            w1=pltpu.make_async_copy(w1_hbm, w1, sem_w.at[1]),
            wq=pltpu.make_async_copy(wqkv_hbm.at[:, pl.ds(0, D)], wq, sem_w.at[2]),
            wv=pltpu.make_async_copy(wqkv_hbm.at[:, pl.ds(2 * D, D)], wv, sem_w.at[3]),
            wo=pltpu.make_async_copy(wo_hbm, wo, sem_w.at[4]),
            w2=pltpu.make_async_copy(w2_hbm, w2, sem_w.at[5]),
            w3=pltpu.make_async_copy(w3_hbm, w3, sem_w.at[6]),
            w4=pltpu.make_async_copy(w4_hbm, w5.at[pl.ds(D, F), :], sem_w.at[7]),
        )
        wcopies["gw"].start()
        xcopy(0).start()

        hbuf[:, 0:PAD, :] = jnp.zeros((5, PAD, 128), f32)
        hbuf[:, PAD + S:PAD + S + PAD, :] = jnp.zeros((5, PAD, 128), f32)

        def p1_pre(r0, n):
            xf = ax[pl.ds(r0, n), :].astype(f32)
            gw = gwv[...].reshape(1, D).astype(f32)
            ln1 = _ln(xf).astype(bf16)
            g = jax.nn.sigmoid(jnp.sum(xf * gw, axis=-1, keepdims=True))
            return ln1, g

        def p1_h(r0, n, ln1):
            return _dot(ln1, w1[...])

        def p1_gate_store(r0, n, g):
            gb = jnp.broadcast_to(g, (n, 128))
            gcol[pl.ds(r0, n), :] = gb
            grow[:, pl.ds(r0, n)] = gb.T[0:8, :]

        def p1_pk(k):
            n = k.shape[0]
            pk = _phi(k)
            zs = jnp.sum(pk.reshape(n // 8, 8, D), axis=0)
            pkb = pk.astype(bf16)
            return zs, [pkb[j * 128:(j + 1) * 128, :].T for j in range(n // 128)]

        def p1_P(r0, n, zs, pkTs, first):
            pkT = jnp.concatenate(pkTs, axis=1)
            xa = ax[pl.ds(r0, n), :]
            if first:
                zacc[...] = zs
                P[...] = _dot(pkT, xa)
            else:
                zacc[...] += zs
                P[...] += _dot(pkT, xa)

        def p1_hstore(r0, n, hpre):
            h = _gelu_scaled(hpre, 0.5)
            for t in range(5):
                hbuf[t, pl.ds(r0 + PAD, n), :] = h[:, t * 128:(t + 1) * 128]

        def phase1_pair(i):
            ra = pl.multiple_of(i * BM, BM)
            rb = pl.multiple_of(i * BM + BM, BM)
            ka = _dot(ax[pl.ds(ra, BM), :], wk[...])
            lna, ga = p1_pre(ra, BM)
            ha = p1_h(ra, BM, lna)
            p1_gate_store(ra, BM, ga)
            zsa, pa = p1_pk(ka)
            kb = _dot(ax[pl.ds(rb, BM), :], wk[...])
            p1_hstore(ra, BM, ha)
            lnb, gb = p1_pre(rb, BM)
            hb = p1_h(rb, BM, lnb)
            p1_gate_store(rb, BM, gb)
            zsb, pb = p1_pk(kb)
            p1_P(ra, 2 * BM, zsa + zsb, pa + pb, False)
            p1_hstore(rb, BM, hb)

        with scope("wait_gw"):
            wcopies["gw"].wait()
        wkcopy.start()
        with scope("wait_x0"):
            xcopy(0).wait()
        xcopy(1).start()
        with scope("B0"):
            lna, ga = p1_pre(0, BM)
            p1_gate_store(0, BM, ga)
        with scope("wait_wk"):
            wkcopy.wait()
        wcopies["w1"].start()
        with scope("B1"):
            ka = _dot(ax[0:BM, :], wk[...])
        with scope("wait_x1"):
            xcopy(1).wait()
        for i in range(PEEL, NB):
            xcopy(i).start()
        with scope("B1b"):
            kb = _dot(ax[BM:2 * BM, :], wk[...])
            zsa, pa = p1_pk(ka)
        with scope("wait_w1"):
            wcopies["w1"].wait()
        for n in ("wq", "wv", "wo", "w2", "w3", "w4"):
            wcopies[n].start()
        with scope("B2"):
            ha = p1_h(0, BM, lna)
            lnb, gb = p1_pre(BM, BM)
            hb = p1_h(BM, BM, lnb)
            p1_gate_store(BM, BM, gb)
            zsb, pb = p1_pk(kb)
            p1_hstore(0, BM, ha)
            p1_P(0, 2 * BM, zsa + zsb, pa + pb, True)
            p1_hstore(BM, BM, hb)

        def p1s(i, c):
            with scope("p1_iter"):
                for u in range(2):
                    xcopy(PEEL + i * 2 + u).wait()
                phase1_pair(PEEL + i * 2)
                return c
        lax.fori_loop(0, (NB - PEEL) // 2, p1s, 0)

        with scope("wait_mid"):
            for n in ("wv", "wo", "wq", "w2", "w3", "w4"):
                wcopies[n].wait()
        with scope("middle"):
            kvs = []
            for t in range(5):
                lo, hi = LO[t], HI[t]
                kvt = _dot(P[lo:hi, :].astype(bf16), wv[:, t * 128:(t + 1) * 128])
                rh = (lax.broadcasted_iota(jnp.int32, (hi - lo, 128), 0) + lo) // DH
                ch = (lax.broadcasted_iota(jnp.int32, (hi - lo, 128), 1) + t * 128) // DH
                kvs.append(jnp.where(rh == ch, kvt, 0.0).astype(bf16))
            wqT[...] = wq[...].T
            z = jnp.sum(zacc[...], axis=0, keepdims=True)
            zb[...] = jnp.broadcast_to(z, (128, D)).T
            ms = [_dot(kvs[t], wo[t * 128:(t + 1) * 128, :]) for t in range(5)]
            for t in range(5):
                lo, hi = LO[t], HI[t]
                a0 = lo if t == 0 else HI[t - 1]
                a1 = hi if t == 4 else LO[t + 1]
                w5[a0:a1, :] = ms[t][a0 - lo:a1 - lo, :].astype(bf16)
                if t < 4:
                    b0, b1 = LO[t + 1], hi
                    w5[b0:b1, :] = (ms[t][b0 - lo:b1 - lo, :] + ms[t + 1][0:b1 - b0, :]).astype(bf16)

        def ocopy(i):
            return pltpu.make_async_copy(obuf.at[pl.ds(i * BM, BM), :], out_hbm.at[0, pl.ds(i * BM, BM), :], sem_o.at[i, 0])

        def ocopy_t(i, t):
            return pltpu.make_async_copy(obuf.at[pl.ds(i * BM, BM), pl.ds(t * 128, 128)],
                                         out_hbm.at[0, pl.ds(i * BM, BM), pl.ds(t * 128, 128)], sem_o.at[i, t])

        def phase2(i, split):
            r0 = pl.multiple_of(i * BM, BM)
            xa = ax[pl.ds(r0, BM), :]

            def hload(t, off):
                return hbuf[t, pl.ds(r0 + PAD + off, BM), :]
            lane = lax.broadcasted_iota(jnp.int32, (BM, 128), 1)
            s0 = hload(0, -1)
            s1 = jnp.where(lane < 32, hload(1, -1), hload(1, 1))
            s2 = jnp.where(lane < 64, hload(2, 1), hload(2, -2))
            s3 = jnp.where(lane < 96, hload(3, -2), hload(3, 2))
            s4 = hload(4, 2)
            hsft = jnp.concatenate([s0, s1, s2, s3, s4], axis=1).astype(bf16)
            xf = xa.astype(f32)
            omg = 1.0 - gcol[pl.ds(r0, BM), :]
            gT = grow[:, pl.ds(r0, BM)]

            qT = _dot_nt(wqT[...], xa)
            hs = _dot(hsft, w2[...])

            pqT = _phi(qT)
            zbv = zb[...]
            zfull = jnp.concatenate([zbv] * (BM // 128), axis=1)
            prod = (pqT * zfull).reshape(H // 2, 40, BM)
            sub = lax.broadcasted_iota(jnp.int32, (H // 2, 40, BM), 1)
            denA = jnp.sum(jnp.where(sub < 20, prod, 0.0), axis=1, keepdims=True) + 1e-6
            denB = jnp.sum(jnp.where(sub >= 20, prod, 0.0), axis=1, keepdims=True) + 1e-6
            g1 = gT[0:1, :].reshape(1, 1, BM)
            rden = jnp.where(sub < 20, g1 / denA, g1 / denB)
            pqsT = (pqT.reshape(H // 2, 40, BM) * rden).reshape(D, BM)
            pqs = pqsT.astype(bf16).T

            x1 = xf + hs
            a = jnp.concatenate([omg] * 5, axis=1) * x1 + _dot(pqs, w5[0:D, :])
            ln2 = _ln(x1).astype(bf16)
            if FREM:
                FM = F - 64
                tremT = _dot_nt(w3[FM:F, :], ln2)
                tpre = _dot_nt(ln2, w3[0:FM, :])
                trem = _gelu_scaled(tremT, 0.5 - 0.5 * gT[0:1, :]).astype(bf16).T
                tmain = _gelu_scaled(tpre, jnp.concatenate([0.5 * omg] * (FM // 128), axis=1)).astype(bf16)
                t = jnp.concatenate([tmain, trem], axis=1)
            else:
                tpre = _dot_nt(ln2, w3[...])
                t = _gelu_scaled(tpre, jnp.concatenate([0.5 * omg] * 14, axis=1)[:, :F]).astype(bf16)
            if split:
                for n in range(5):
                    cols = slice(n * 128, (n + 1) * 128)
                    obuf[pl.ds(r0, BM), cols] = (a[:, cols] + _dot(t, w5[D:D + F, cols])).astype(bf16)
                    ocopy_t(i, n).start()
            else:
                obuf[pl.ds(r0, BM), :] = (a + _dot(t, w5[D:D + F, :])).astype(bf16)
                ocopy(i).start()

        def is_split(u):
            return SPLIT_OUT and u == UN2 - 1

        def p2s(i, c):
            with scope("p2_iter"):
                for u in range(UN2):
                    phase2(i * UN2 + u, is_split(u))
                return c
        lax.fori_loop(0, NB // UN2, p2s, 0)
        with scope("wait_out"):
            for i in range(NB):
                if is_split(i % UN2):
                    for n in range(5):
                        ocopy_t(i, n).wait()
                else:
                    ocopy(i).wait()

    @jax.jit
    def run(A_x, A_wqkv, A_wo, B_x, B_w1, B_w2, B_w3, B_w4, gate_w):
        hbm = pl.BlockSpec(memory_space=pltpu.HBM)
        return pl.pallas_call(
            kernel,
            out_shape=jax.ShapeDtypeStruct((1, S, D), bf16),
            in_specs=[hbm] * 9,
            out_specs=hbm,
            scratch_shapes=[
                pltpu.VMEM((S, D), bf16),
                pltpu.VMEM((D, D), bf16), pltpu.VMEM((D, D), bf16), pltpu.VMEM((D, D), bf16), pltpu.VMEM((D, D), bf16),
                pltpu.VMEM((D, D), bf16), pltpu.VMEM((D, D), bf16), pltpu.VMEM((F, D), bf16), pltpu.VMEM((D + F, D), bf16),
                pltpu.VMEM((D,), bf16),
                pltpu.VMEM((D, D), bf16),
                pltpu.VMEM((D, D), f32), pltpu.VMEM((8, D), f32), pltpu.VMEM((D, 128), f32),
                pltpu.VMEM((5, S + 2 * PAD, 128), f32), pltpu.VMEM((S, D), bf16),
                pltpu.VMEM((S, 128), f32), pltpu.VMEM((8, S), f32),
                pltpu.SemaphoreType.DMA((NB,)), pltpu.SemaphoreType.DMA((1,)),
                pltpu.SemaphoreType.DMA((8,)), pltpu.SemaphoreType.DMA((NB, 5)),
            ],
            compiler_params=pltpu.CompilerParams(vmem_limit_bytes=100 * 1024 * 1024),
            name="gated_mix",
        )(A_x, A_wqkv, A_wo, B_x, B_w1, B_w2, B_w3.T, B_w4, gate_w)
    return run


_run = make()


def pallas_gated_mix__linear_attn_block__mixer_s_mlp__prompt_kernel(A_x, A_wqkv, A_wo, B_x, B_w1, B_w2, B_w3, B_w4, gate_w):
    return _run(A_x, A_wqkv, A_wo, B_x, B_w1, B_w2, B_w3, B_w4, gate_w)
```

```python
import contextlib
import jax
import jax.numpy as jnp
from jax import lax
import jax.experimental.pallas as pl
import jax.experimental.pallas.tpu as pltpu

S, D, F, H = 2048, 640, 1728, 32
DH = D // H
NT = (((1,), (1,)), ((), ()))
f32 = jnp.float32
bf16 = jnp.bfloat16
LO = (0, 112, 240, 368, 496)
HI = (144, 272, 400, 528, 640)


def _phi(t):
    return jnp.where(t > 0, t + 1.0, jnp.exp(t)) + 1e-6


def _ln(x):
    m = jnp.mean(x, axis=-1, keepdims=True)
    xc = x - m
    v = jnp.mean(xc * xc, axis=-1, keepdims=True)
    rs = lax.rsqrt(v + 1e-5)
    return x * rs - m * rs


def _gelu_scaled(x, half):
    c = 0.7978845608028654
    inner = x * (c + (c * 0.044715) * (x * x))
    return (half * x) * (1.0 + jnp.tanh(inner))


def _dot(a, b):
    return jnp.dot(a, b, preferred_element_type=f32)


def _dot_nt(a, b):
    return lax.dot_general(a, b, NT, preferred_element_type=f32)


def make(BM=256, PAD=8, UN2=2, SPLIT_OUT=True, NA=384, RSPLIT=False, INTER=False, scopes=False):
    NB = S // BM
    PEEL = 2

    def scope(name):
        return jax.named_scope(name) if scopes else contextlib.nullcontext()

    def kernel(ax_hbm, wqkv_hbm, wo_hbm, bx_hbm, w1_hbm, w2_hbm, w3_hbm, w4_hbm, gw_hbm,
               out_hbm,
               ax, wq, wk, wv, wo, w1, w2, w3, w5, gwv,
               wqT, P, zacc, zb, hbuf, obuf, gcol, grow, w2b,
               sem_ax, sem_wk, sem_w, sem_o):
        def xcopy(i):
            return pltpu.make_async_copy(ax_hbm.at[0, pl.ds(i * BM, BM), :], ax.at[pl.ds(i * BM, BM), :], sem_ax.at[i])

        wka = pltpu.make_async_copy(wqkv_hbm.at[:, pl.ds(D, NA)], wk.at[:, pl.ds(0, NA)], sem_wk.at[0])
        wkb = pltpu.make_async_copy(wqkv_hbm.at[:, pl.ds(D + NA, D - NA)], wk.at[:, pl.ds(NA, D - NA)], sem_wk.at[1])

        wcopies = dict(
            gw=pltpu.make_async_copy(gw_hbm, gwv, sem_w.at[0]),
            w1=pltpu.make_async_copy(w1_hbm, w1, sem_w.at[1]),
            wq=pltpu.make_async_copy(wqkv_hbm.at[:, pl.ds(0, D)], wq, sem_w.at[2]),
            wv=pltpu.make_async_copy(wqkv_hbm.at[:, pl.ds(2 * D, D)], wv, sem_w.at[3]),
            wo=pltpu.make_async_copy(wo_hbm, wo, sem_w.at[4]),
            w2=pltpu.make_async_copy(w2_hbm, w2, sem_w.at[5]),
            w3=pltpu.make_async_copy(w3_hbm, w3, sem_w.at[6]),
            w4=pltpu.make_async_copy(w4_hbm, w5.at[pl.ds(D, F), :], sem_w.at[7]),
        )
        wcopies["gw"].start()
        xcopy(0).start()

        hbuf[:, 0:PAD, :] = jnp.zeros((5, PAD, 128), f32)
        hbuf[:, PAD + S:PAD + S + PAD, :] = jnp.zeros((5, PAD, 128), f32)

        def p1_pre(r0, n):
            xf = ax[pl.ds(r0, n), :].astype(f32)
            gw = gwv[...].reshape(1, D).astype(f32)
            ln1 = _ln(xf).astype(bf16)
            g = jax.nn.sigmoid(jnp.sum(xf * gw, axis=-1, keepdims=True))
            return ln1, g

        def p1_h(r0, n, ln1):
            return _dot(ln1, w1[...])

        def p1_gate_store(r0, n, g):
            gb = jnp.broadcast_to(g, (n, 128))
            gcol[pl.ds(r0, n), :] = gb
            grow[:, pl.ds(r0, n)] = gb.T[0:8, :]

        def p1_pk(k):
            n = k.shape[0]
            pk = _phi(k)
            zs = jnp.sum(pk.reshape(n // 8, 8, D), axis=0)
            pkb = pk.astype(bf16)
            return zs, [pkb[j * 128:(j + 1) * 128, :].T for j in range(n // 128)]

        def p1_P(r0, n, zs, pkTs, first):
            pkT = jnp.concatenate(pkTs, axis=1)
            xa = ax[pl.ds(r0, n), :]
            if first:
                zacc[...] = zs
                P[...] = _dot(pkT, xa)
            else:
                zacc[...] += zs
                P[...] += _dot(pkT, xa)

        def p1_hstore(r0, n, hpre):
            h = _gelu_scaled(hpre, 0.5)
            for t in range(5):
                hbuf[t, pl.ds(r0 + PAD, n), :] = h[:, t * 128:(t + 1) * 128]

        def phase1_pair(i):
            ra = pl.multiple_of(i * BM, BM)
            rb = pl.multiple_of(i * BM + BM, BM)
            ka = _dot(ax[pl.ds(ra, BM), :], wk[...])
            lna, ga = p1_pre(ra, BM)
            ha = p1_h(ra, BM, lna)
            p1_gate_store(ra, BM, ga)
            zsa, pa = p1_pk(ka)
            kb = _dot(ax[pl.ds(rb, BM), :], wk[...])
            p1_hstore(ra, BM, ha)
            lnb, gb = p1_pre(rb, BM)
            hb = p1_h(rb, BM, lnb)
            p1_gate_store(rb, BM, gb)
            zsb, pb = p1_pk(kb)
            p1_P(ra, 2 * BM, zsa + zsb, pa + pb, False)
            p1_hstore(rb, BM, hb)

        with scope("wait_gw"):
            wcopies["gw"].wait()
        wka.start()
        with scope("wait_x0"):
            xcopy(0).wait()
        wkb.start()
        with scope("B0"):
            lna, ga = p1_pre(0, BM)
            p1_gate_store(0, BM, ga)
        with scope("wait_wka"):
            wka.wait()
        xcopy(1).start()
        with scope("B1a"):
            ka0 = _dot(ax[0:BM, :], wk[:, 0:NA])
        with scope("wait_wkb"):
            wkb.wait()
            xcopy(1).wait()
        wcopies["w1"].start()
        with scope("B1b"):
            ka1 = _dot(ax[0:BM, :], wk[:, NA:D])
            kb = _dot(ax[BM:2 * BM, :], wk[...])
            zsa, pa = p1_pk(jnp.concatenate([ka0, ka1], axis=1))
        with scope("wait_w1"):
            wcopies["w1"].wait()
        for i in range(PEEL, NB):
            xcopy(i).start()
        with scope("B2"):
            ha = p1_h(0, BM, lna)
            lnb, gb = p1_pre(BM, BM)
            zsb, pb = p1_pk(kb)
            hb = p1_h(BM, BM, lnb)
            p1_hstore(0, BM, ha)
            p1_gate_store(BM, BM, gb)
            p1_P(0, 2 * BM, zsa + zsb, pa + pb, True)
            p1_hstore(BM, BM, hb)

        with scope("wait_x23"):
            xcopy(PEEL).wait()
        for n in ("wq", "wv", "wo", "w2", "w3", "w4"):
            wcopies[n].start()

        def p1s(i, c):
            with scope("p1_iter"):
                @pl.when(i > 0)
                def _():
                    xcopy(PEEL + i * 2).wait()
                xcopy(PEEL + i * 2 + 1).wait()
                phase1_pair(PEEL + i * 2)
                return c
        lax.fori_loop(0, (NB - PEEL) // 2, p1s, 0)

        with scope("wait_mid"):
            for n in ("wv", "wo", "wq", "w2", "w3", "w4"):
                wcopies[n].wait()
        with scope("middle"):
            kvs = []
            for t in range(5):
                lo, hi = LO[t], HI[t]
                kvt = _dot(P[lo:hi, :].astype(bf16), wv[:, t * 128:(t + 1) * 128])
                rh = (lax.broadcasted_iota(jnp.int32, (hi - lo, 128), 0) + lo) // DH
                ch = (lax.broadcasted_iota(jnp.int32, (hi - lo, 128), 1) + t * 128) // DH
                kvs.append(jnp.where(rh == ch, kvt, 0.0).astype(bf16))
            wqT[...] = wq[...].T
            z = jnp.sum(zacc[...], axis=0, keepdims=True)
            zb[...] = jnp.broadcast_to(z, (128, D)).T
            w2m = jnp.mean(w2[...].astype(f32), axis=1, keepdims=True)
            w2b[...] = jnp.broadcast_to(w2m, (D, 128)).T[0:8, :]
            ms = [_dot(kvs[t], wo[t * 128:(t + 1) * 128, :]) for t in range(5)]
            for t in range(5):
                lo, hi = LO[t], HI[t]
                a0 = lo if t == 0 else HI[t - 1]
                a1 = hi if t == 4 else LO[t + 1]
                w5[a0:a1, :] = ms[t][a0 - lo:a1 - lo, :].astype(bf16)
                if t < 4:
                    b0, b1 = LO[t + 1], hi
                    w5[b0:b1, :] = (ms[t][b0 - lo:b1 - lo, :] + ms[t + 1][0:b1 - b0, :]).astype(bf16)

        def ocopy(i):
            return pltpu.make_async_copy(obuf.at[pl.ds(i * BM, BM), :], out_hbm.at[0, pl.ds(i * BM, BM), :], sem_o.at[i, 0])

        def ocopy_t(i, t):
            return pltpu.make_async_copy(obuf.at[pl.ds(i * BM, BM), pl.ds(t * 128, 128)],
                                         out_hbm.at[0, pl.ds(i * BM, BM), pl.ds(t * 128, 128)], sem_o.at[i, t])

        FM = F - 64

        def p2_front(i):
            r0 = pl.multiple_of(i * BM, BM)
            xa = ax[pl.ds(r0, BM), :]

            def hload(t, off):
                return hbuf[t, pl.ds(r0 + PAD + off, BM), :]
            lane = lax.broadcasted_iota(jnp.int32, (BM, 128), 1)
            s0 = hload(0, -1)
            s1 = jnp.where(lane < 32, hload(1, -1), hload(1, 1))
            s2 = jnp.where(lane < 64, hload(2, 1), hload(2, -2))
            s3 = jnp.where(lane < 96, hload(3, -2), hload(3, 2))
            s4 = hload(4, 2)
            hsf = jnp.concatenate([s0, s1, s2, s3, s4], axis=1)
            hsft = hsf.astype(bf16)
            xf = xa.astype(f32)
            m = jnp.sum(xf * (1.0 / D) + hsf * w2b[0:1, :], axis=-1, keepdims=True)
            omg = 1.0 - gcol[pl.ds(r0, BM), :]
            gT = grow[:, pl.ds(r0, BM)]

            qT = _dot_nt(wqT[...], xa)
            hs = _dot(hsft, w2[...])

            pqT = _phi(qT)
            zbv = zb[...]
            zfull = jnp.concatenate([zbv] * (BM // 128), axis=1)
            prod = (pqT * zfull).reshape(H // 2, 40, BM)
            sub = lax.broadcasted_iota(jnp.int32, (H // 2, 40, BM), 1)
            denA = jnp.sum(jnp.where(sub < 20, prod, 0.0), axis=1, keepdims=True) + 1e-6
            denB = jnp.sum(jnp.where(sub >= 20, prod, 0.0), axis=1, keepdims=True) + 1e-6
            g1 = gT[0:1, :].reshape(1, 1, BM)
            rden = jnp.where(sub < 20, g1 / denA, g1 / denB)
            pqsT = (pqT.reshape(H // 2, 40, BM) * rden).reshape(D, BM)
            pqs = pqsT.astype(bf16).T
            xc = ((xf - m) + hs).astype(bf16)
            return xc, m, pqs, omg, gT

        def p2_mid(ln2, m, pqs, omg, gT):
            xr = ln2.astype(f32)
            a = jnp.concatenate([omg] * 5, axis=1) * (xr + m) + _dot(pqs, w5[0:D, :])
            rs = lax.rsqrt(jnp.mean(xr * xr, axis=-1, keepdims=True) + 1e-5)
            rsb = jnp.broadcast_to(rs, (BM, 128))
            rsT = rsb.T[0:1, :]
            half = jnp.concatenate([0.5 * omg] * (FM // 128), axis=1)
            rsf = jnp.concatenate([rsb] * (FM // 128), axis=1)
            if RSPLIT:
                hb = BM // 2
                t0 = _gelu_scaled(_dot_nt(ln2[0:hb], w3[0:FM, :]) * rsf[0:hb], half[0:hb]).astype(bf16)
                tremT = _dot_nt(w3[FM:F, :], ln2)
                t1 = _gelu_scaled(_dot_nt(ln2[hb:BM], w3[0:FM, :]) * rsf[hb:BM], half[hb:BM]).astype(bf16)
                tmain = jnp.concatenate([t0, t1], axis=0)
            else:
                tremT = _dot_nt(w3[FM:F, :], ln2)
                tmain = _gelu_scaled(_dot_nt(ln2, w3[0:FM, :]) * rsf, half).astype(bf16)
            trem = _gelu_scaled(tremT * rsT, 0.5 - 0.5 * gT[0:1, :]).astype(bf16).T
            return a, jnp.concatenate([tmain, trem], axis=1)

        def p2_back(i, a, t, split):
            r0 = pl.multiple_of(i * BM, BM)
            if split:
                for n in range(5):
                    cols = slice(n * 128, (n + 1) * 128)
                    obuf[pl.ds(r0, BM), cols] = (a[:, cols] + _dot(t, w5[D:D + F, cols])).astype(bf16)
                    ocopy_t(i, n).start()
            else:
                obuf[pl.ds(r0, BM), :] = (a + _dot(t, w5[D:D + F, :])).astype(bf16)
                ocopy(i).start()

        def p2_pair(i):
            fa = p2_front(i)
            a_a, t_a = p2_mid(*fa)
            if INTER:
                fb = p2_front(i + 1)
                p2_back(i, a_a, t_a, False)
            else:
                p2_back(i, a_a, t_a, False)
                fb = p2_front(i + 1)
            a_b, t_b = p2_mid(*fb)
            p2_back(i + 1, a_b, t_b, SPLIT_OUT)

        def is_split(u):
            return SPLIT_OUT and u == UN2 - 1

        def p2s(i, c):
            with scope("p2_iter"):
                p2_pair(i * 2)
                return c
        lax.fori_loop(0, NB // UN2, p2s, 0)
        with scope("wait_out"):
            for i in range(NB):
                if is_split(i % UN2):
                    for n in range(5):
                        ocopy_t(i, n).wait()
                else:
                    ocopy(i).wait()

    @jax.jit
    def run(A_x, A_wqkv, A_wo, B_x, B_w1, B_w2, B_w3, B_w4, gate_w):
        hbm = pl.BlockSpec(memory_space=pltpu.HBM)
        return pl.pallas_call(
            kernel,
            out_shape=jax.ShapeDtypeStruct((1, S, D), bf16),
            in_specs=[hbm] * 9,
            out_specs=hbm,
            scratch_shapes=[
                pltpu.VMEM((S, D), bf16),
                pltpu.VMEM((D, D), bf16), pltpu.VMEM((D, D), bf16), pltpu.VMEM((D, D), bf16), pltpu.VMEM((D, D), bf16),
                pltpu.VMEM((D, D), bf16), pltpu.VMEM((D, D), bf16), pltpu.VMEM((F, D), bf16), pltpu.VMEM((D + F, D), bf16),
                pltpu.VMEM((D,), bf16),
                pltpu.VMEM((D, D), bf16),
                pltpu.VMEM((D, D), f32), pltpu.VMEM((8, D), f32), pltpu.VMEM((D, 128), f32),
                pltpu.VMEM((5, S + 2 * PAD, 128), f32), pltpu.VMEM((S, D), bf16),
                pltpu.VMEM((S, 128), f32), pltpu.VMEM((8, S), f32), pltpu.VMEM((8, D), f32),
                pltpu.SemaphoreType.DMA((NB,)), pltpu.SemaphoreType.DMA((2,)),
                pltpu.SemaphoreType.DMA((8,)), pltpu.SemaphoreType.DMA((NB, 5)),
            ],
            compiler_params=pltpu.CompilerParams(vmem_limit_bytes=100 * 1024 * 1024),
            name="gated_mix",
        )(A_x, A_wqkv, A_wo, B_x, B_w1, B_w2, B_w3.T, B_w4, gate_w)
    return run


_run = make(RSPLIT=True, INTER=True)


def pallas_gated_mix__linear_attn_block__mixer_s_mlp__prompt_kernel(A_x, A_wqkv, A_wo, B_x, B_w1, B_w2, B_w3, B_w4, gate_w):
    return _run(A_x, A_wqkv, A_wo, B_x, B_w1, B_w2, B_w3, B_w4, gate_w)
```

```python
import contextlib
import jax
import jax.numpy as jnp
from jax import lax
import jax.experimental.pallas as pl
import jax.experimental.pallas.tpu as pltpu

S, D, F, H = 2048, 640, 1728, 32
DH = D // H
NT = (((1,), (1,)), ((), ()))
f32 = jnp.float32
bf16 = jnp.bfloat16
LO = (0, 112, 240, 368, 496)
HI = (144, 272, 400, 528, 640)


def _phi(t):
    return jnp.where(t > 0, t + 1.0, jnp.exp(t)) + 1e-6


def _ln(x):
    m = jnp.mean(x, axis=-1, keepdims=True)
    xc = x - m
    v = jnp.mean(xc * xc, axis=-1, keepdims=True)
    rs = lax.rsqrt(v + 1e-5)
    return x * rs - m * rs


def _gelu_scaled(x, half):
    c = 0.7978845608028654
    inner = x * (c + (c * 0.044715) * (x * x))
    return (half * x) * (1.0 + jnp.tanh(inner))


def _dot(a, b):
    return jnp.dot(a, b, preferred_element_type=f32)


def _dot_nt(a, b):
    return lax.dot_general(a, b, NT, preferred_element_type=f32)


def make(BM=256, PAD=8, UN2=2, SPLIT_OUT=True, NA=384, RSPLIT=False, INTER=False, B2V=0, BQ=256, PAIR=True, scopes=False):
    NB = S // BM
    NQ = S // BQ
    PEEL = 2

    def scope(name):
        return jax.named_scope(name) if scopes else contextlib.nullcontext()

    def kernel(ax_hbm, wqkv_hbm, wo_hbm, bx_hbm, w1_hbm, w2_hbm, w3_hbm, w4_hbm, gw_hbm,
               out_hbm,
               ax, wq, wk, wv, wo, w1, w2, w3, w5, gwv,
               wqT, P, zacc, zb, hbuf, obuf, gcol, grow, w2b, hpart,
               sem_ax, sem_wk, sem_w, sem_o):
        def xcopy(i):
            return pltpu.make_async_copy(ax_hbm.at[0, pl.ds(i * BM, BM), :], ax.at[pl.ds(i * BM, BM), :], sem_ax.at[i])

        wkcopy = pltpu.make_async_copy(wqkv_hbm.at[:, pl.ds(D, D)], wk, sem_wk.at[0])
        w1a = pltpu.make_async_copy(w1_hbm.at[pl.ds(0, NA), :], w1.at[pl.ds(0, NA), :], sem_wk.at[1])
        w1b = pltpu.make_async_copy(w1_hbm.at[pl.ds(NA, D - NA), :], w1.at[pl.ds(NA, D - NA), :], sem_wk.at[2])

        wcopies = dict(
            gw=pltpu.make_async_copy(gw_hbm, gwv, sem_w.at[0]),
            wq=pltpu.make_async_copy(wqkv_hbm.at[:, pl.ds(0, D)], wq, sem_w.at[2]),
            wv=pltpu.make_async_copy(wqkv_hbm.at[:, pl.ds(2 * D, D)], wv, sem_w.at[3]),
            wo=pltpu.make_async_copy(wo_hbm, wo, sem_w.at[4]),
            w2=pltpu.make_async_copy(w2_hbm, w2, sem_w.at[5]),
            w3=pltpu.make_async_copy(w3_hbm, w3, sem_w.at[6]),
            w4=pltpu.make_async_copy(w4_hbm, w5.at[pl.ds(D, F), :], sem_w.at[7]),
        )
        wcopies["gw"].start()
        xcopy(0).start()

        hbuf[:, 0:PAD, :] = jnp.zeros((5, PAD, 128), f32)
        hbuf[:, PAD + S:PAD + S + PAD, :] = jnp.zeros((5, PAD, 128), f32)

        def p1_ln(r0, n):
            return _ln(ax[pl.ds(r0, n), :].astype(f32)).astype(bf16)

        def p1_gate(r0, n):
            xf = ax[pl.ds(r0, n), :].astype(f32)
            gw = gwv[...].reshape(1, D).astype(f32)
            return jax.nn.sigmoid(jnp.sum(xf * gw, axis=-1, keepdims=True))

        def p1_pre(r0, n):
            return p1_ln(r0, n), p1_gate(r0, n)

        def p1_h(r0, n, ln1):
            return _dot(ln1, w1[...])

        def p1_gate_store(r0, n, g):
            gb = jnp.broadcast_to(g, (n, 128))
            gcol[pl.ds(r0, n), :] = gb
            grow[:, pl.ds(r0, n)] = gb.T[0:8, :]

        def p1_pk(k):
            n = k.shape[0]
            pk = _phi(k)
            zs = jnp.sum(pk.reshape(n // 8, 8, D), axis=0)
            pkb = pk.astype(bf16)
            return zs, [pkb[j * 128:(j + 1) * 128, :].T for j in range(n // 128)]

        def p1_P(r0, n, zs, pkTs, first):
            pkT = jnp.concatenate(pkTs, axis=1)
            xa = ax[pl.ds(r0, n), :]
            if first:
                zacc[...] = zs
                P[...] = _dot(pkT, xa)
            else:
                zacc[...] += zs
                P[...] += _dot(pkT, xa)

        def p1_hstore(r0, n, hpre):
            h = _gelu_scaled(hpre, 0.5)
            for t in range(5):
                hbuf[t, pl.ds(r0 + PAD, n), :] = h[:, t * 128:(t + 1) * 128]

        def phase1_pair(i):
            ra = pl.multiple_of(i * BM, BM)
            rb = pl.multiple_of(i * BM + BM, BM)
            ka = _dot(ax[pl.ds(ra, BM), :], wk[...])
            lna, ga = p1_pre(ra, BM)
            ha = p1_h(ra, BM, lna)
            p1_gate_store(ra, BM, ga)
            zsa, pa = p1_pk(ka)
            kb = _dot(ax[pl.ds(rb, BM), :], wk[...])
            p1_hstore(ra, BM, ha)
            lnb, gb = p1_pre(rb, BM)
            hb = p1_h(rb, BM, lnb)
            p1_gate_store(rb, BM, gb)
            zsb, pb = p1_pk(kb)
            p1_P(ra, 2 * BM, zsa + zsb, pa + pb, False)
            p1_hstore(rb, BM, hb)

        with scope("wait_gw"):
            wcopies["gw"].wait()
        w1a.start()
        with scope("wait_x0"):
            xcopy(0).wait()
        w1b.start()
        with scope("B0"):
            lna, ga = p1_pre(0, BM)
            p1_gate_store(0, BM, ga)
        with scope("wait_w1a"):
            w1a.wait()
        xcopy(1).start()
        with scope("B1a"):
            hpart[...] = _dot(lna[:, 0:NA], w1[0:NA, :])
        with scope("wait_w1b"):
            w1b.wait()
            xcopy(1).wait()
        wkcopy.start()
        with scope("B1b"):
            ha = hpart[...] + _dot(lna[:, NA:D], w1[NA:D, :])
            lnb, gb = p1_pre(BM, BM)
            hb = p1_h(BM, BM, lnb)
            p1_hstore(0, BM, ha)
            p1_gate_store(BM, BM, gb)
            p1_hstore(BM, BM, hb)
        with scope("wait_wk"):
            wkcopy.wait()
        for i in range(PEEL, NB):
            xcopy(i).start()
        with scope("B2"):
            ka = _dot(ax[0:BM, :], wk[...])
            kb = _dot(ax[BM:2 * BM, :], wk[...])
            zsa, pa = p1_pk(ka)
            Pa = _dot(jnp.concatenate(pa, axis=1), ax[0:BM, :])
            zsb, pb = p1_pk(kb)
            zacc[...] = zsa + zsb
            P[...] = Pa + _dot(jnp.concatenate(pb, axis=1), ax[BM:2 * BM, :])

        with scope("wait_x23"):
            xcopy(PEEL).wait()
        for n in ("wq", "wv", "wo", "w2", "w3", "w4"):
            wcopies[n].start()

        def p1s(i, c):
            with scope("p1_iter"):
                @pl.when(i > 0)
                def _():
                    xcopy(PEEL + i * 2).wait()
                xcopy(PEEL + i * 2 + 1).wait()
                phase1_pair(PEEL + i * 2)
                return c
        lax.fori_loop(0, (NB - PEEL) // 2, p1s, 0)

        with scope("wait_mid"):
            for n in ("wv", "wo", "wq", "w2", "w3", "w4"):
                wcopies[n].wait()
        with scope("middle"):
            kvs = []
            for t in range(5):
                lo, hi = LO[t], HI[t]
                kvt = _dot(P[lo:hi, :].astype(bf16), wv[:, t * 128:(t + 1) * 128])
                rh = (lax.broadcasted_iota(jnp.int32, (hi - lo, 128), 0) + lo) // DH
                ch = (lax.broadcasted_iota(jnp.int32, (hi - lo, 128), 1) + t * 128) // DH
                kvs.append(jnp.where(rh == ch, kvt, 0.0).astype(bf16))
            wqT[...] = wq[...].T
            z = jnp.sum(zacc[...], axis=0, keepdims=True)
            zb[...] = jnp.broadcast_to(z, (128, D)).T
            w2m = jnp.mean(w2[...].astype(f32), axis=1, keepdims=True)
            w2b[...] = jnp.broadcast_to(w2m, (D, 128)).T[0:8, :]
            ms = [_dot(kvs[t], wo[t * 128:(t + 1) * 128, :]) for t in range(5)]
            for t in range(5):
                lo, hi = LO[t], HI[t]
                a0 = lo if t == 0 else HI[t - 1]
                a1 = hi if t == 4 else LO[t + 1]
                w5[a0:a1, :] = ms[t][a0 - lo:a1 - lo, :].astype(bf16)
                if t < 4:
                    b0, b1 = LO[t + 1], hi
                    w5[b0:b1, :] = (ms[t][b0 - lo:b1 - lo, :] + ms[t + 1][0:b1 - b0, :]).astype(bf16)

        def ocopy(i):
            return pltpu.make_async_copy(obuf.at[pl.ds(i * BQ, BQ), :], out_hbm.at[0, pl.ds(i * BQ, BQ), :], sem_o.at[i, 0])

        def ocopy_t(i, t):
            c = min(t, 4)
            r0, n = (i * BQ, BQ) if t < 4 else (i * BQ + (t - 4) * (BQ // 2), BQ // 2)
            return pltpu.make_async_copy(obuf.at[pl.ds(r0, n), pl.ds(c * 128, 128)],
                                         out_hbm.at[0, pl.ds(r0, n), pl.ds(c * 128, 128)], sem_o.at[i, t])

        FM = F - 64

        def p2_front(i):
            r0 = pl.multiple_of(i * BQ, BQ)
            xa = ax[pl.ds(r0, BQ), :]

            def hload(t, off):
                return hbuf[t, pl.ds(r0 + PAD + off, BQ), :]
            lane = lax.broadcasted_iota(jnp.int32, (BQ, 128), 1)
            s0 = hload(0, -1)
            s1 = jnp.where(lane < 32, hload(1, -1), hload(1, 1))
            s2 = jnp.where(lane < 64, hload(2, 1), hload(2, -2))
            s3 = jnp.where(lane < 96, hload(3, -2), hload(3, 2))
            s4 = hload(4, 2)
            hsf = jnp.concatenate([s0, s1, s2, s3, s4], axis=1)
            hsft = hsf.astype(bf16)
            xf = xa.astype(f32)
            m = jnp.sum(xf * (1.0 / D) + hsf * w2b[0:1, :], axis=-1, keepdims=True)
            omg = 1.0 - gcol[pl.ds(r0, BQ), :]
            gT = grow[:, pl.ds(r0, BQ)]

            qT = _dot_nt(wqT[...], xa)
            hs = _dot(hsft, w2[...])

            pqT = _phi(qT)
            zbv = zb[...]
            zfull = jnp.concatenate([zbv] * (BQ // 128), axis=1)
            prod = (pqT * zfull).reshape(H // 2, 40, BQ)
            sub = lax.broadcasted_iota(jnp.int32, (H // 2, 40, BQ), 1)
            denA = jnp.sum(jnp.where(sub < 20, prod, 0.0), axis=1, keepdims=True) + 1e-6
            denB = jnp.sum(jnp.where(sub >= 20, prod, 0.0), axis=1, keepdims=True) + 1e-6
            g1 = gT[0:1, :].reshape(1, 1, BQ)
            rden = jnp.where(sub < 20, g1 / denA, g1 / denB)
            pqsT = (pqT.reshape(H // 2, 40, BQ) * rden).reshape(D, BQ)
            pqs = pqsT.astype(bf16).T
            xc = ((xf - m) + hs).astype(bf16)
            return xc, m, pqs, omg, gT

        def p2_mid(ln2, m, pqs, omg, gT):
            xr = ln2.astype(f32)
            a = jnp.concatenate([omg] * 5, axis=1) * (xr + m) + _dot(pqs, w5[0:D, :])
            rs = lax.rsqrt(jnp.mean(xr * xr, axis=-1, keepdims=True) + 1e-5)
            rsb = jnp.broadcast_to(rs, (BQ, 128))
            rsT = rsb.T[0:1, :]
            half = jnp.concatenate([0.5 * omg] * (FM // 128), axis=1)
            rsf = jnp.concatenate([rsb] * (FM // 128), axis=1)
            if RSPLIT:
                hb = BQ // 2
                t0 = _gelu_scaled(_dot_nt(ln2[0:hb], w3[0:FM, :]) * rsf[0:hb], half[0:hb]).astype(bf16)
                tremT = _dot_nt(w3[FM:F, :], ln2)
                t1 = _gelu_scaled(_dot_nt(ln2[hb:BQ], w3[0:FM, :]) * rsf[hb:BQ], half[hb:BQ]).astype(bf16)
                tmain = jnp.concatenate([t0, t1], axis=0)
            else:
                tremT = _dot_nt(w3[FM:F, :], ln2)
                tmain = _gelu_scaled(_dot_nt(ln2, w3[0:FM, :]) * rsf, half).astype(bf16)
            trem = _gelu_scaled(tremT * rsT, 0.5 - 0.5 * gT[0:1, :]).astype(bf16).T
            return a, jnp.concatenate([tmain, trem], axis=1)

        def p2_back(i, a, t, split):
            r0 = pl.multiple_of(i * BQ, BQ)
            if split:
                for n in range(5):
                    cols = slice(n * 128, (n + 1) * 128)
                    res = (a[:, cols] + _dot(t, w5[D:D + F, cols])).astype(bf16)
                    if n < 4:
                        obuf[pl.ds(r0, BQ), cols] = res
                        ocopy_t(i, n).start()
                    else:
                        hq = BQ // 2
                        obuf[pl.ds(r0, hq), cols] = res[0:hq]
                        ocopy_t(i, 4).start()
                        obuf[pl.ds(r0 + hq, hq), cols] = res[hq:BQ]
                        ocopy_t(i, 5).start()
            else:
                obuf[pl.ds(r0, BQ), :] = (a + _dot(t, w5[D:D + F, :])).astype(bf16)
                ocopy(i).start()

        def p2_pair(i):
            fa = p2_front(i)
            a_a, t_a = p2_mid(*fa)
            if INTER:
                fb = p2_front(i + 1)
                p2_back(i, a_a, t_a, False)
            else:
                p2_back(i, a_a, t_a, False)
                fb = p2_front(i + 1)
            a_b, t_b = p2_mid(*fb)
            p2_back(i + 1, a_b, t_b, SPLIT_OUT)

        def p2_single(i):
            fa = p2_front(i)
            a_a, t_a = p2_mid(*fa)
            p2_back(i, a_a, t_a, SPLIT_OUT)

        def is_split(u):
            return SPLIT_OUT and u == UN2 - 1

        def p2s(i, c):
            with scope("p2_iter"):
                p2_pair(i * 2) if PAIR else p2_single(i)
                return c
        lax.fori_loop(0, NQ // (2 if PAIR else 1), p2s, 0)
        with scope("wait_out"):
            for i in range(NQ):
                if SPLIT_OUT and ((not PAIR) or i % 2 == 1):
                    for n in range(6):
                        ocopy_t(i, n).wait()
                else:
                    ocopy(i).wait()

    @jax.jit
    def run(A_x, A_wqkv, A_wo, B_x, B_w1, B_w2, B_w3, B_w4, gate_w):
        hbm = pl.BlockSpec(memory_space=pltpu.HBM)
        return pl.pallas_call(
            kernel,
            out_shape=jax.ShapeDtypeStruct((1, S, D), bf16),
            in_specs=[hbm] * 9,
            out_specs=hbm,
            scratch_shapes=[
                pltpu.VMEM((S, D), bf16),
                pltpu.VMEM((D, D), bf16), pltpu.VMEM((D, D), bf16), pltpu.VMEM((D, D), bf16), pltpu.VMEM((D, D), bf16),
                pltpu.VMEM((D, D), bf16), pltpu.VMEM((D, D), bf16), pltpu.VMEM((F, D), bf16), pltpu.VMEM((D + F, D), bf16),
                pltpu.VMEM((D,), bf16),
                pltpu.VMEM((D, D), bf16),
                pltpu.VMEM((D, D), f32), pltpu.VMEM((8, D), f32), pltpu.VMEM((D, 128), f32),
                pltpu.VMEM((5, S + 2 * PAD, 128), f32), pltpu.VMEM((S, D), bf16),
                pltpu.VMEM((S, 128), f32), pltpu.VMEM((8, S), f32), pltpu.VMEM((8, D), f32), pltpu.VMEM((BM, D), f32),
                pltpu.SemaphoreType.DMA((NB,)), pltpu.SemaphoreType.DMA((3,)),
                pltpu.SemaphoreType.DMA((8,)), pltpu.SemaphoreType.DMA((NQ, 6)),
            ],
            compiler_params=pltpu.CompilerParams(vmem_limit_bytes=100 * 1024 * 1024),
            name="gated_mix",
        )(A_x, A_wqkv, A_wo, B_x, B_w1, B_w2, B_w3.T, B_w4, gate_w)
    return run


_run = make(RSPLIT=True, BQ=512, PAIR=False, NA=384)


def pallas_gated_mix__linear_attn_block__mixer_s_mlp__prompt_kernel(A_x, A_wqkv, A_wo, B_x, B_w1, B_w2, B_w3, B_w4, gate_w):
    return _run(A_x, A_wqkv, A_wo, B_x, B_w1, B_w2, B_w3, B_w4, gate_w)
```

```python
import jax
import jax.numpy as jnp
from jax import lax
import jax.experimental.pallas as pl
import jax.experimental.pallas.tpu as pltpu

S, D, F, H = 2048, 640, 1728, 32
DH = D // H
BM = 256
BQ = 512
NB = S // BM
NQ = S // BQ
PAD = 8
NA = 384
FM = F - 64
LO = (0, 112, 240, 368, 496)
HI = (144, 272, 400, 528, 640)
NT = (((1,), (1,)), ((), ()))
f32 = jnp.float32
bf16 = jnp.bfloat16


def _phi(t):
    return jnp.where(t > 0, t + 1.0, jnp.exp(t)) + 1e-6


def _ln(x):
    m = jnp.mean(x, axis=-1, keepdims=True)
    xc = x - m
    v = jnp.mean(xc * xc, axis=-1, keepdims=True)
    rs = lax.rsqrt(v + 1e-5)
    return x * rs - m * rs


def _gelu_scaled(x, half):
    c = 0.7978845608028654
    inner = x * (c + (c * 0.044715) * (x * x))
    return (half * x) * (1.0 + jnp.tanh(inner))


def _dot(a, b):
    return jnp.dot(a, b, preferred_element_type=f32)


def _dot_nt(a, b):
    return lax.dot_general(a, b, NT, preferred_element_type=f32)


def _kernel(ax_hbm, wqkv_hbm, wo_hbm, bx_hbm, w1_hbm, w2_hbm, w3_hbm, w4_hbm, gw_hbm,
            out_hbm,
            ax, wq, wk, wv, wo, w1, w2, w3, w5, gwv,
            wqT, P, zacc, zb, hbuf, obuf, gcol, grow, w2b, hpart,
            sem_x, sem_a, sem_w, sem_o):
    del bx_hbm

    def xcopy(i):
        return pltpu.make_async_copy(ax_hbm.at[0, pl.ds(i * BM, BM), :], ax.at[pl.ds(i * BM, BM), :], sem_x.at[i])

    gwc = pltpu.make_async_copy(gw_hbm, gwv, sem_a.at[0])
    w1a = pltpu.make_async_copy(w1_hbm.at[pl.ds(0, NA), :], w1.at[pl.ds(0, NA), :], sem_a.at[1])
    w1b = pltpu.make_async_copy(w1_hbm.at[pl.ds(NA, D - NA), :], w1.at[pl.ds(NA, D - NA), :], sem_a.at[2])
    wkc = pltpu.make_async_copy(wqkv_hbm.at[:, pl.ds(D, D)], wk, sem_a.at[3])
    late = [
        pltpu.make_async_copy(wqkv_hbm.at[:, pl.ds(0, D)], wq, sem_w.at[0]),
        pltpu.make_async_copy(wqkv_hbm.at[:, pl.ds(2 * D, D)], wv, sem_w.at[1]),
        pltpu.make_async_copy(wo_hbm, wo, sem_w.at[2]),
        pltpu.make_async_copy(w2_hbm, w2, sem_w.at[3]),
        pltpu.make_async_copy(w3_hbm, w3, sem_w.at[4]),
        pltpu.make_async_copy(w4_hbm, w5.at[pl.ds(D, F), :], sem_w.at[5]),
    ]
    gwc.start()
    xcopy(0).start()

    hbuf[:, 0:PAD, :] = jnp.zeros((5, PAD, 128), f32)
    hbuf[:, PAD + S:PAD + S + PAD, :] = jnp.zeros((5, PAD, 128), f32)

    def p1_pre(r0):
        xf = ax[pl.ds(r0, BM), :].astype(f32)
        gw = gwv[...].reshape(1, D).astype(f32)
        g = jax.nn.sigmoid(jnp.sum(xf * gw, axis=-1, keepdims=True))
        return _ln(xf).astype(bf16), g

    def p1_gate_store(r0, g):
        gb = jnp.broadcast_to(g, (BM, 128))
        gcol[pl.ds(r0, BM), :] = gb
        grow[:, pl.ds(r0, BM)] = gb.T[0:8, :]

    def p1_pk(k):
        pk = _phi(k)
        zs = jnp.sum(pk.reshape(BM // 8, 8, D), axis=0)
        pkb = pk.astype(bf16)
        return zs, [pkb[j * 128:(j + 1) * 128, :].T for j in range(BM // 128)]

    def p1_hstore(r0, hpre):
        h = _gelu_scaled(hpre, 0.5)
        for t in range(5):
            hbuf[t, pl.ds(r0 + PAD, BM), :] = h[:, t * 128:(t + 1) * 128]

    def phase1_pair(i):
        ra = pl.multiple_of(i * BM, BM)
        rb = pl.multiple_of(i * BM + BM, BM)
        ka = _dot(ax[pl.ds(ra, BM), :], wk[...])
        lna, ga = p1_pre(ra)
        ha = _dot(lna, w1[...])
        p1_gate_store(ra, ga)
        zsa, pa = p1_pk(ka)
        kb = _dot(ax[pl.ds(rb, BM), :], wk[...])
        p1_hstore(ra, ha)
        lnb, gb = p1_pre(rb)
        hb = _dot(lnb, w1[...])
        p1_gate_store(rb, gb)
        zsb, pb = p1_pk(kb)
        zacc[...] += zsa + zsb
        P[...] += _dot(jnp.concatenate(pa + pb, axis=1), ax[pl.ds(ra, 2 * BM), :])
        p1_hstore(rb, hb)

    gwc.wait()
    w1a.start()
    xcopy(0).wait()
    w1b.start()
    lna, ga = p1_pre(0)
    p1_gate_store(0, ga)
    w1a.wait()
    xcopy(1).start()
    hpart[...] = _dot(lna[:, 0:NA], w1[0:NA, :])
    w1b.wait()
    xcopy(1).wait()
    wkc.start()
    ha = hpart[...] + _dot(lna[:, NA:D], w1[NA:D, :])
    lnb, gb = p1_pre(BM)
    hb = _dot(lnb, w1[...])
    p1_hstore(0, ha)
    p1_gate_store(BM, gb)
    p1_hstore(BM, hb)
    wkc.wait()
    for i in range(2, NB):
        xcopy(i).start()
    ka = _dot(ax[0:BM, :], wk[...])
    kb = _dot(ax[BM:2 * BM, :], wk[...])
    zsa, pa = p1_pk(ka)
    pa_x = _dot(jnp.concatenate(pa, axis=1), ax[0:BM, :])
    zsb, pb = p1_pk(kb)
    zacc[...] = zsa + zsb
    P[...] = pa_x + _dot(jnp.concatenate(pb, axis=1), ax[BM:2 * BM, :])
    xcopy(2).wait()
    for c in late:
        c.start()

    def p1_step(i, carry):
        @pl.when(i > 0)
        def _():
            xcopy(2 + i * 2).wait()
        xcopy(3 + i * 2).wait()
        phase1_pair(2 + i * 2)
        return carry
    lax.fori_loop(0, (NB - 2) // 2, p1_step, 0)

    for c in late:
        c.wait()
    kvs = []
    for t in range(5):
        lo, hi = LO[t], HI[t]
        kvt = _dot(P[lo:hi, :].astype(bf16), wv[:, t * 128:(t + 1) * 128])
        rh = (lax.broadcasted_iota(jnp.int32, (hi - lo, 128), 0) + lo) // DH
        ch = (lax.broadcasted_iota(jnp.int32, (hi - lo, 128), 1) + t * 128) // DH
        kvs.append(jnp.where(rh == ch, kvt, 0.0).astype(bf16))
    wqT[...] = wq[...].T
    z = jnp.sum(zacc[...], axis=0, keepdims=True)
    zb[...] = jnp.broadcast_to(z, (128, D)).T
    w2m = jnp.mean(w2[...].astype(f32), axis=1, keepdims=True)
    w2b[...] = jnp.broadcast_to(w2m, (D, 128)).T[0:8, :]
    ms = [_dot(kvs[t], wo[t * 128:(t + 1) * 128, :]) for t in range(5)]
    for t in range(5):
        lo, hi = LO[t], HI[t]
        a0 = lo if t == 0 else HI[t - 1]
        a1 = hi if t == 4 else LO[t + 1]
        w5[a0:a1, :] = ms[t][a0 - lo:a1 - lo, :].astype(bf16)
        if t < 4:
            b0, b1 = LO[t + 1], hi
            w5[b0:b1, :] = (ms[t][b0 - lo:b1 - lo, :] + ms[t + 1][0:b1 - b0, :]).astype(bf16)

    def ocopy(i, t):
        c = min(t, 4)
        r0, n = (i * BQ, BQ) if t < 4 else (i * BQ + (t - 4) * (BQ // 2), BQ // 2)
        return pltpu.make_async_copy(obuf.at[pl.ds(r0, n), pl.ds(c * 128, 128)],
                                     out_hbm.at[0, pl.ds(r0, n), pl.ds(c * 128, 128)], sem_o.at[i * 6 + t])

    def p2_step(i, carry):
        r0 = pl.multiple_of(i * BQ, BQ)
        xa = ax[pl.ds(r0, BQ), :]

        def hload(t, off):
            return hbuf[t, pl.ds(r0 + PAD + off, BQ), :]
        lane = lax.broadcasted_iota(jnp.int32, (BQ, 128), 1)
        s0 = hload(0, -1)
        s1 = jnp.where(lane < 32, hload(1, -1), hload(1, 1))
        s2 = jnp.where(lane < 64, hload(2, 1), hload(2, -2))
        s3 = jnp.where(lane < 96, hload(3, -2), hload(3, 2))
        s4 = hload(4, 2)
        hsf = jnp.concatenate([s0, s1, s2, s3, s4], axis=1)
        hsft = hsf.astype(bf16)
        xf = xa.astype(f32)
        m = jnp.sum(xf * (1.0 / D) + hsf * w2b[0:1, :], axis=-1, keepdims=True)
        omg = 1.0 - gcol[pl.ds(r0, BQ), :]
        gT = grow[:, pl.ds(r0, BQ)]

        qT = _dot_nt(wqT[...], xa)
        hs = _dot(hsft, w2[...])

        pqT = _phi(qT)
        zfull = jnp.concatenate([zb[...]] * (BQ // 128), axis=1)
        prod = (pqT * zfull).reshape(H // 2, 40, BQ)
        sub = lax.broadcasted_iota(jnp.int32, (H // 2, 40, BQ), 1)
        den_a = jnp.sum(jnp.where(sub < 20, prod, 0.0), axis=1, keepdims=True) + 1e-6
        den_b = jnp.sum(jnp.where(sub >= 20, prod, 0.0), axis=1, keepdims=True) + 1e-6
        g1 = gT[0:1, :].reshape(1, 1, BQ)
        rden = jnp.where(sub < 20, g1 / den_a, g1 / den_b)
        pqs = (pqT.reshape(H // 2, 40, BQ) * rden).reshape(D, BQ).astype(bf16).T

        xc = ((xf - m) + hs).astype(bf16)
        xr = xc.astype(f32)
        acc = jnp.concatenate([omg] * 5, axis=1) * (xr + m) + _dot(pqs, w5[0:D, :])
        rs = lax.rsqrt(jnp.mean(xr * xr, axis=-1, keepdims=True) + 1e-5)
        rsb = jnp.broadcast_to(rs, (BQ, 128))
        rsT = rsb.T[0:1, :]
        half = jnp.concatenate([0.5 * omg] * (FM // 128), axis=1)
        rsf = jnp.concatenate([rsb] * (FM // 128), axis=1)
        hq = BQ // 2
        t0 = _gelu_scaled(_dot_nt(xc[0:hq], w3[0:FM, :]) * rsf[0:hq], half[0:hq]).astype(bf16)
        tremT = _dot_nt(w3[FM:F, :], xc)
        t1 = _gelu_scaled(_dot_nt(xc[hq:BQ], w3[0:FM, :]) * rsf[hq:BQ], half[hq:BQ]).astype(bf16)
        trem = _gelu_scaled(tremT * rsT, 0.5 - 0.5 * gT[0:1, :]).astype(bf16).T
        t = jnp.concatenate([jnp.concatenate([t0, t1], axis=0), trem], axis=1)

        for n in range(5):
            cols = slice(n * 128, (n + 1) * 128)
            res = (acc[:, cols] + _dot(t, w5[D:D + F, cols])).astype(bf16)
            if n < 4:
                obuf[pl.ds(r0, BQ), cols] = res
                ocopy(i, n).start()
            else:
                obuf[pl.ds(r0, hq), cols] = res[0:hq]
                ocopy(i, 4).start()
                obuf[pl.ds(r0 + hq, hq), cols] = res[hq:BQ]
                ocopy(i, 5).start()
        return carry
    lax.fori_loop(0, NQ, p2_step, 0)
    for i in range(NQ):
        for t in range(6):
            ocopy(i, t).wait()


@jax.jit
def pallas_gated_mix__linear_attn_block__mixer_s_mlp__prompt_kernel(
    A_x: jax.Array,
    A_wqkv: jax.Array,
    A_wo: jax.Array,
    B_x: jax.Array,
    B_w1: jax.Array,
    B_w2: jax.Array,
    B_w3: jax.Array,
    B_w4: jax.Array,
    gate_w: jax.Array,
):
    hbm = pl.BlockSpec(memory_space=pltpu.MemorySpace.HBM)
    return pl.pallas_call(
        _kernel,
        out_shape=jax.ShapeDtypeStruct((1, S, D), bf16),
        in_specs=[hbm] * 9,
        out_specs=hbm,
        scratch_shapes=[
            pltpu.VMEM((S, D), bf16),
            pltpu.VMEM((D, D), bf16), pltpu.VMEM((D, D), bf16),
            pltpu.VMEM((D, D), bf16), pltpu.VMEM((D, D), bf16),
            pltpu.VMEM((D, D), bf16), pltpu.VMEM((D, D), bf16),
            pltpu.VMEM((F, D), bf16), pltpu.VMEM((D + F, D), bf16),
            pltpu.VMEM((D,), bf16),
            pltpu.VMEM((D, D), bf16),
            pltpu.VMEM((D, D), f32), pltpu.VMEM((8, D), f32),
            pltpu.VMEM((D, 128), f32),
            pltpu.VMEM((5, S + 2 * PAD, 128), f32),
            pltpu.VMEM((S, D), bf16),
            pltpu.VMEM((S, 128), f32), pltpu.VMEM((8, S), f32),
            pltpu.VMEM((8, D), f32), pltpu.VMEM((BM, D), f32),
            pltpu.SemaphoreType.DMA((NB,)), pltpu.SemaphoreType.DMA((4,)),
            pltpu.SemaphoreType.DMA((6,)), pltpu.SemaphoreType.DMA((NQ * 6,)),
        ],
        compiler_params=pltpu.CompilerParams(vmem_limit_bytes=100 * 1024 * 1024),
        name="gated_mix",
    )(A_x, A_wqkv, A_wo, B_x, B_w1, B_w2, B_w3.T, B_w4, gate_w)
```

```python
import jax
import jax.numpy as jnp
from jax import lax
import jax.experimental.pallas as pl
import jax.experimental.pallas.tpu as pltpu

S, D, F, H = 2048, 640, 1728, 32
DH = D // H
BM = 256
BQ = 512
NB = S // BM
NQ = S // BQ
PAD = 8
NA = 384
FM = F - 64
LO = (0, 112, 240, 368, 496)
HI = (144, 272, 400, 528, 640)
NT = (((1,), (1,)), ((), ()))
f32 = jnp.float32
bf16 = jnp.bfloat16


def _phi(t):
    return jnp.where(t > 0, t + 1.0, jnp.exp(t)) + 1e-6


def _ln(x):
    m = jnp.mean(x, axis=-1, keepdims=True)
    xc = x - m
    v = jnp.mean(xc * xc, axis=-1, keepdims=True)
    rs = lax.rsqrt(v + 1e-5)
    return x * rs - m * rs


def _gelu_scaled(x, half):
    c = 0.7978845608028654
    inner = x * (c + (c * 0.044715) * (x * x))
    return (half * x) * (1.0 + jnp.tanh(inner))


def _dot(a, b):
    return jnp.dot(a, b, preferred_element_type=f32)


def _dot_nt(a, b):
    return lax.dot_general(a, b, NT, preferred_element_type=f32)


def _kernel(ax_hbm, wqkv_hbm, wo_hbm, bx_hbm, w1_hbm, w2_hbm, w3_hbm, w4_hbm, gw_hbm,
            out_hbm,
            ax, wq, wk, wv, wo, w1, w2, w3, w5, gwv,
            wqT, P, zacc, zb, hbuf, obuf, gcol, grow, w2b, hpart,
            sems):
    del bx_hbm

    def xcopy(i, sem):
        return pltpu.make_async_copy(ax_hbm.at[0, pl.ds(i * BM, BM), :], ax.at[pl.ds(i * BM, BM), :], sem)

    gwc = pltpu.make_async_copy(gw_hbm, gwv, sems.at[0])
    x0c = xcopy(0, sems.at[1])
    w1a = pltpu.make_async_copy(w1_hbm.at[pl.ds(0, NA), :], w1.at[pl.ds(0, NA), :], sems.at[0])
    w1b = pltpu.make_async_copy(w1_hbm.at[pl.ds(NA, D - NA), :], w1.at[pl.ds(NA, D - NA), :], sems.at[1])
    x1c = xcopy(1, sems.at[0])
    wkc = pltpu.make_async_copy(wqkv_hbm.at[:, pl.ds(D, D)], wk, sems.at[1])
    xrest = [xcopy(i, sems.at[0]) for i in range(2, NB)]
    late = [
        pltpu.make_async_copy(wqkv_hbm.at[:, pl.ds(0, D)], wq, sems.at[0]),
        pltpu.make_async_copy(wqkv_hbm.at[:, pl.ds(2 * D, D)], wv, sems.at[0]),
        pltpu.make_async_copy(wo_hbm, wo, sems.at[0]),
        pltpu.make_async_copy(w2_hbm, w2, sems.at[0]),
        pltpu.make_async_copy(w3_hbm, w3, sems.at[0]),
        pltpu.make_async_copy(w4_hbm, w5.at[pl.ds(D, F), :], sems.at[0]),
    ]
    gwc.start()
    x0c.start()

    hbuf[:, 0:PAD, :] = jnp.zeros((5, PAD, 128), f32)
    hbuf[:, PAD + S:PAD + S + PAD, :] = jnp.zeros((5, PAD, 128), f32)

    def p1_pre(r0):
        xf = ax[pl.ds(r0, BM), :].astype(f32)
        gw = gwv[...].reshape(1, D).astype(f32)
        g = jax.nn.sigmoid(jnp.sum(xf * gw, axis=-1, keepdims=True))
        return _ln(xf).astype(bf16), g

    def p1_gate_store(r0, g):
        gb = jnp.broadcast_to(g, (BM, 128))
        gcol[pl.ds(r0, BM), :] = gb
        grow[:, pl.ds(r0, BM)] = gb.T[0:8, :]

    def p1_pk(k):
        pk = _phi(k)
        zs = jnp.sum(pk.reshape(BM // 8, 8, D), axis=0)
        pkb = pk.astype(bf16)
        return zs, [pkb[j * 128:(j + 1) * 128, :].T for j in range(BM // 128)]

    def p1_hstore(r0, hpre):
        h = _gelu_scaled(hpre, 0.5)
        for t in range(5):
            hbuf[t, pl.ds(r0 + PAD, BM), :] = h[:, t * 128:(t + 1) * 128]

    def phase1_pair(i):
        ra = pl.multiple_of(i * BM, BM)
        rb = pl.multiple_of(i * BM + BM, BM)
        ka = _dot(ax[pl.ds(ra, BM), :], wk[...])
        lna, ga = p1_pre(ra)
        ha = _dot(lna, w1[...])
        p1_gate_store(ra, ga)
        zsa, pa = p1_pk(ka)
        kb = _dot(ax[pl.ds(rb, BM), :], wk[...])
        p1_hstore(ra, ha)
        lnb, gb = p1_pre(rb)
        hb = _dot(lnb, w1[...])
        p1_gate_store(rb, gb)
        zsb, pb = p1_pk(kb)
        zacc[...] += zsa + zsb
        P[...] += _dot(jnp.concatenate(pa + pb, axis=1), ax[pl.ds(ra, 2 * BM), :])
        p1_hstore(rb, hb)

    gwc.wait()
    w1a.start()
    x0c.wait()
    w1b.start()
    lna, ga = p1_pre(0)
    p1_gate_store(0, ga)
    w1a.wait()
    x1c.start()
    hpart[...] = _dot(lna[:, 0:NA], w1[0:NA, :])
    w1b.wait()
    x1c.wait()
    wkc.start()
    ha = hpart[...] + _dot(lna[:, NA:D], w1[NA:D, :])
    lnb, gb = p1_pre(BM)
    hb = _dot(lnb, w1[...])
    p1_hstore(0, ha)
    p1_gate_store(BM, gb)
    p1_hstore(BM, hb)
    wkc.wait()
    for c in xrest:
        c.start()
    ka = _dot(ax[0:BM, :], wk[...])
    kb = _dot(ax[BM:2 * BM, :], wk[...])
    zsa, pa = p1_pk(ka)
    pa_x = _dot(jnp.concatenate(pa, axis=1), ax[0:BM, :])
    zsb, pb = p1_pk(kb)
    zacc[...] = zsa + zsb
    P[...] = pa_x + _dot(jnp.concatenate(pb, axis=1), ax[BM:2 * BM, :])
    for c in xrest:
        c.wait()
    for c in late:
        c.start()

    def p1_step(i, carry):
        phase1_pair(2 + i * 2)
        return carry
    lax.fori_loop(0, (NB - 2) // 2, p1_step, 0)

    for c in late:
        c.wait()
    kvs = []
    for t in range(5):
        lo, hi = LO[t], HI[t]
        kvt = _dot(P[lo:hi, :].astype(bf16), wv[:, t * 128:(t + 1) * 128])
        rh = (lax.broadcasted_iota(jnp.int32, (hi - lo, 128), 0) + lo) // DH
        ch = (lax.broadcasted_iota(jnp.int32, (hi - lo, 128), 1) + t * 128) // DH
        kvs.append(jnp.where(rh == ch, kvt, 0.0).astype(bf16))
    wqT[...] = wq[...].T
    z = jnp.sum(zacc[...], axis=0, keepdims=True)
    zb[...] = jnp.broadcast_to(z, (128, D)).T
    w2m = jnp.mean(w2[...].astype(f32), axis=1, keepdims=True)
    w2b[...] = jnp.broadcast_to(w2m, (D, 128)).T[0:8, :]
    ms = [_dot(kvs[t], wo[t * 128:(t + 1) * 128, :]) for t in range(5)]
    for t in range(5):
        lo, hi = LO[t], HI[t]
        a0 = lo if t == 0 else HI[t - 1]
        a1 = hi if t == 4 else LO[t + 1]
        w5[a0:a1, :] = ms[t][a0 - lo:a1 - lo, :].astype(bf16)
        if t < 4:
            b0, b1 = LO[t + 1], hi
            w5[b0:b1, :] = (ms[t][b0 - lo:b1 - lo, :] + ms[t + 1][0:b1 - b0, :]).astype(bf16)

    def ocopy(i, t):
        c = min(t, 4)
        r0, n = (i * BQ, BQ) if t < 4 else (i * BQ + (t - 4) * (BQ // 2), BQ // 2)
        return pltpu.make_async_copy(obuf.at[pl.ds(r0, n), pl.ds(c * 128, 128)],
                                     out_hbm.at[0, pl.ds(r0, n), pl.ds(c * 128, 128)], sems.at[1])

    def p2_step(i, carry):
        r0 = pl.multiple_of(i * BQ, BQ)
        xa = ax[pl.ds(r0, BQ), :]

        def hload(t, off):
            return hbuf[t, pl.ds(r0 + PAD + off, BQ), :]
        lane = lax.broadcasted_iota(jnp.int32, (BQ, 128), 1)
        s0 = hload(0, -1)
        s1 = jnp.where(lane < 32, hload(1, -1), hload(1, 1))
        s2 = jnp.where(lane < 64, hload(2, 1), hload(2, -2))
        s3 = jnp.where(lane < 96, hload(3, -2), hload(3, 2))
        s4 = hload(4, 2)
        hsf = jnp.concatenate([s0, s1, s2, s3, s4], axis=1)
        hsft = hsf.astype(bf16)
        xf = xa.astype(f32)
        m = jnp.sum(xf * (1.0 / D) + hsf * w2b[0:1, :], axis=-1, keepdims=True)
        omg = 1.0 - gcol[pl.ds(r0, BQ), :]
        gT = grow[:, pl.ds(r0, BQ)]

        qT = _dot_nt(wqT[...], xa)
        hs = _dot(hsft, w2[...])

        pqT = _phi(qT)
        zfull = jnp.concatenate([zb[...]] * (BQ // 128), axis=1)
        prod = (pqT * zfull).reshape(H // 2, 40, BQ)
        sub = lax.broadcasted_iota(jnp.int32, (H // 2, 40, BQ), 1)
        den_a = jnp.sum(jnp.where(sub < 20, prod, 0.0), axis=1, keepdims=True) + 1e-6
        den_b = jnp.sum(jnp.where(sub >= 20, prod, 0.0), axis=1, keepdims=True) + 1e-6
        g1 = gT[0:1, :].reshape(1, 1, BQ)
        rden = jnp.where(sub < 20, g1 / den_a, g1 / den_b)
        pqs = (pqT.reshape(H // 2, 40, BQ) * rden).reshape(D, BQ).astype(bf16).T

        xc = ((xf - m) + hs).astype(bf16)
        xr = xc.astype(f32)
        acc = jnp.concatenate([omg] * 5, axis=1) * (xr + m) + _dot(pqs, w5[0:D, :])
        rs = lax.rsqrt(jnp.mean(xr * xr, axis=-1, keepdims=True) + 1e-5)
        rsb = jnp.broadcast_to(rs, (BQ, 128))
        rsT = rsb.T[0:1, :]
        half = jnp.concatenate([0.5 * omg] * (FM // 128), axis=1)
        rsf = jnp.concatenate([rsb] * (FM // 128), axis=1)
        hq = BQ // 2
        t0 = _gelu_scaled(_dot_nt(xc[0:hq], w3[0:FM, :]) * rsf[0:hq], half[0:hq]).astype(bf16)
        tremT = _dot_nt(w3[FM:F, :], xc)
        t1 = _gelu_scaled(_dot_nt(xc[hq:BQ], w3[0:FM, :]) * rsf[hq:BQ], half[hq:BQ]).astype(bf16)
        trem = _gelu_scaled(tremT * rsT, 0.5 - 0.5 * gT[0:1, :]).astype(bf16).T
        t = jnp.concatenate([jnp.concatenate([t0, t1], axis=0), trem], axis=1)

        for n in range(5):
            cols = slice(n * 128, (n + 1) * 128)
            res = (acc[:, cols] + _dot(t, w5[D:D + F, cols])).astype(bf16)
            if n < 4:
                obuf[pl.ds(r0, BQ), cols] = res
                ocopy(i, n).start()
            else:
                obuf[pl.ds(r0, hq), cols] = res[0:hq]
                ocopy(i, 4).start()
                obuf[pl.ds(r0 + hq, hq), cols] = res[hq:BQ]
                ocopy(i, 5).start()
        return carry
    lax.fori_loop(0, NQ, p2_step, 0)
    for i in range(NQ):
        for t in range(6):
            ocopy(i, t).wait()


@jax.jit
def pallas_gated_mix__linear_attn_block__mixer_s_mlp__prompt_kernel(
    A_x: jax.Array,
    A_wqkv: jax.Array,
    A_wo: jax.Array,
    B_x: jax.Array,
    B_w1: jax.Array,
    B_w2: jax.Array,
    B_w3: jax.Array,
    B_w4: jax.Array,
    gate_w: jax.Array,
):
    hbm = pl.BlockSpec(memory_space=pltpu.MemorySpace.HBM)
    return pl.pallas_call(
        _kernel,
        out_shape=jax.ShapeDtypeStruct((1, S, D), bf16),
        in_specs=[hbm] * 9,
        out_specs=hbm,
        scratch_shapes=[
            pltpu.VMEM((S, D), bf16),
            pltpu.VMEM((D, D), bf16), pltpu.VMEM((D, D), bf16),
            pltpu.VMEM((D, D), bf16), pltpu.VMEM((D, D), bf16),
            pltpu.VMEM((D, D), bf16), pltpu.VMEM((D, D), bf16),
            pltpu.VMEM((F, D), bf16), pltpu.VMEM((D + F, D), bf16),
            pltpu.VMEM((D,), bf16),
            pltpu.VMEM((D, D), bf16),
            pltpu.VMEM((D, D), f32), pltpu.VMEM((8, D), f32),
            pltpu.VMEM((D, 128), f32),
            pltpu.VMEM((5, S + 2 * PAD, 128), f32),
            pltpu.VMEM((S, D), bf16),
            pltpu.VMEM((S, 128), f32), pltpu.VMEM((8, S), f32),
            pltpu.VMEM((8, D), f32), pltpu.VMEM((BM, D), f32),
            pltpu.SemaphoreType.DMA((2,)),
        ],
        compiler_params=pltpu.CompilerParams(vmem_limit_bytes=100 * 1024 * 1024),
        name="gated_mix",
    )(A_x, A_wqkv, A_wo, B_x, B_w1, B_w2, B_w3.T, B_w4, gate_w)
```
